```python
import os as _os
_os.environ.setdefault("JAX_PLATFORMS", "cpu")
import jax
import jax.numpy as jnp

def _softmax(x, axis=-1):
    return jax.nn.softmax(x, axis=axis)
def _gelu(x):
    return jax.nn.gelu(x, approximate=True)
def _silu(x):
    return jax.nn.silu(x)
def _sigmoid(x):
    return jax.nn.sigmoid(x)
def _layernorm(x, axis=-1, eps=1e-5):
    m = jnp.mean(x, axis=axis, keepdims=True)
    v = jnp.var(x, axis=axis, keepdims=True)
    return (x - m) / jnp.sqrt(v + eps)
def _scatter_add(tgt, idx, src, axis=0):
    return tgt.at[idx].add(src)
def _segment_sum(src, seg, n):
    return jax.ops.segment_sum(src, seg, n)
class _Rng:
    def __init__(self, key):
        self._k = key
    def _next(self):
        self._k, sub = jax.random.split(self._k)
        return sub
    def normal(self, shape):
        return jax.random.normal(self._next(), shape, dtype=jnp.bfloat16)
    def randint(self, lo, hi, shape):
        return jax.random.randint(self._next(), shape, lo, hi, dtype=jnp.int32)
    def uniform(self, shape, lo=0.0, hi=1.0):
        return jax.random.uniform(self._next(), shape, jnp.bfloat16, lo, hi)
    def permutation(self, n):
        return jax.random.permutation(self._next(), n)


kernel_name = 'standalone__gqa_block_cached__near_ridge'

def setup_inputs():
    _rng = _Rng(jax.random.key(int.from_bytes(__import__("os").urandom(4), "little")))
    _w = (lambda a: (lambda t: t.astype(jnp.bfloat16) if jnp.issubdtype(t.dtype, jnp.floating) else t)(jnp.asarray(a)))
    B, Sq, D = 8, 80, 512
    Hq, Hkv, Sk, Dh = 32, 8, 2048, 128
    assert Hq % Hkv == 0, (Hq, Hkv)
    return {
        "x": _w((lambda *s: _rng.normal(s) * 0.8)(B, Sq, D)),
        "k_cache": _w((lambda *s: _rng.normal(s) * 0.8)(B, Hkv, Sk, Dh)),
        "v_cache": _w((lambda *s: _rng.normal(s) * 0.05)(B, Hkv, Sk, Dh)),
        "wq": _w((lambda *s: _rng.normal(s) * 0.8)(D, Hq * Dh) * (D ** -0.5)),
        "wo": _w((lambda *s: _rng.normal(s) * 0.05)(Hq * Dh, D) * ((Hq * Dh) ** -0.5)),
    }

def reference(x, k_cache, v_cache, wq, wo):
    B, Sq, D = x.shape
    Hq, Dh = 32, 128
    Hkv = k_cache.shape[1]
    rep = Hq // Hkv
    q = (lambda x, *d: x.transpose(*d))((x @ wq).reshape(B, Sq, Hq, Dh), 0, 2, 1, 3)
    k = jnp.repeat(k_cache, rep, axis=1)
    v = jnp.repeat(v_cache, rep, axis=1)
    scores = jnp.einsum("bhqd,bhkd->bhqk", q, k) * (Dh ** -0.5)
    p = _softmax(scores, axis=-1)
    o = jnp.einsum("bhqk,bhkd->bhqd", p, v)
    return (lambda x, *d: x.transpose(*d))(o, 0, 2, 1, 3).reshape(B, Sq, Hq * Dh) @ wo
```

```python
import functools
import jax
import jax.numpy as jnp
from jax import lax
import jax.experimental.pallas as pl
import jax.experimental.pallas.tpu as pltpu

LOG2E = 1.4426950408889634
CK = 512
NOBC = 1
PHASES = [(1, 1), (1, 1), (1, 1), (1, 1), (2, 4), (4, 3), (8, 5)]
ORDER = 'q,p0,p1,p2,p3,s,k0,k1,k2,k3,m,f,O'.split(',')
LAG = int('s' in ORDER)

F32 = jnp.float32
BF16 = jnp.bfloat16
U32 = jnp.uint32
NT = (((1,), (1,)), ((), ()))


def _kernel(x_hbm, k_hbm, v_hbm, wq_hbm, wo_hbm, out_hbm,
            x_s, wq_s, wo_s, k_s, v_s, q_s, s0, s1, m0, m1, a0, a1, l0, l1, acc_s, out_s,
            sem_x, sem_wq, sem_wo, sem_k, sem_v, sem_o, sem_f,
            *, B, Hkv, Sq, Sk, rep, Dh, qscale):
    N = B * Hkv
    G = rep * Dh
    R = rep * Sq
    sb, mb, ab, lb = (s0, s1), (m0, m1), (a0, a1), (l0, l1)

    def kv_copy(hbm, buf, sem, n0, cnt, i):
        return pltpu.make_async_copy(hbm.at[pl.ds(n0 % B, cnt), n0 // B], buf.at[pl.ds(n0, cnt)], sem.at[i])

    k_copy = functools.partial(kv_copy, k_hbm, k_s, sem_k)
    v_copy = functools.partial(kv_copy, v_hbm, v_s, sem_v)

    def x_copy(b0, cnt):
        return pltpu.make_async_copy(x_hbm.at[pl.ds(b0, cnt)], x_s.at[pl.ds(b0, cnt)], sem_x.at[b0])

    def wq_copy(h):
        return pltpu.make_async_copy(wq_hbm.at[:, pl.ds(pl.multiple_of(h * G, G), G)], wq_s.at[h], sem_wq.at[h])

    def wo_copy(h):
        return pltpu.make_async_copy(wo_hbm.at[pl.ds(pl.multiple_of(h * G, G), G), :], wo_s.at[h], sem_wo.at[h])

    def out_copy(b0, cnt, i):
        return pltpu.make_async_copy(out_s.at[pl.ds(b0, cnt)], out_hbm.at[pl.ds(b0, cnt)], sem_o.at[i])

    def ld(ref, idx, lo, n):
        w = ref.bitcast(U32)[(*idx, slice(lo // 2, (lo + n) // 2), slice(None))]
        return pltpu.bitcast(w, BF16)

    def st(ref, idx, lo, val):
        n = val.shape[0]
        ref.bitcast(U32)[(*idx, slice(lo // 2, (lo + n) // 2), slice(None))] = pltpu.bitcast(val, U32)

    def qproj(n):
        q = jnp.dot(x_s[n % B], wq_s[n // B], preferred_element_type=F32) * qscale
        q = q.astype(BF16)
        for r in range(rep):
            st(q_s, (), r * Sq, q[:, r * Dh:(r + 1) * Dh])

    def qk_chunk(n, par, j, mrun):
        k = ld(k_s, (n,), j * CK, CK)
        s = lax.dot_general(ld(q_s, (), 0, R), k, NT, preferred_element_type=F32)
        sb[par][:, j * CK:(j + 1) * CK] = s
        for t in range(CK // 128):
            sti = s[:, t * 128:(t + 1) * 128]
            mrun = sti if mrun is None else jnp.maximum(mrun, sti)
        return mrun

    def qk_fin(par, mrun):
        m = jnp.max(mrun, axis=1, keepdims=True)
        mb[par][...] = jnp.broadcast_to(m, (R, 128))

    def pv_chunk(n, par, j, carry):
        lrun, acc = carry
        m = mb[par][...]
        ps = []
        for t in range(CK // 128):
            p = jnp.exp2(sb[par][:, j * CK + t * 128:j * CK + (t + 1) * 128] - m)
            lrun = p if lrun is None else lrun + p
            ps.append(p)
        p = jnp.concatenate(ps, axis=1).astype(BF16)
        v = ld(v_s, (n,), j * CK, CK)
        o = jnp.dot(p, v, preferred_element_type=F32)
        acc = o if acc is None else acc + o
        return lrun, acc

    def stash(par, carry):
        lrun, acc = carry
        lb[par][...] = lrun
        ab[par][...] = acc

    def fin(carry):
        lrun, acc = carry
        l = jnp.sum(lrun, axis=1, keepdims=True)
        o = acc * pl.reciprocal(l, full_range=False)
        return jnp.concatenate([o[r * Sq:(r + 1) * Sq] for r in range(rep)], axis=1).astype(BF16)

    def outproj(n, o):
        y = acc_s[n % B] + jnp.dot(o, wo_s[n // B], preferred_element_type=F32)
        acc_s[n % B] = y
        out_s[n % B] = y.astype(BF16)

    def slot(n, par, lo=None, hi=None):
        ok = lambda d: (lo is None or d >= lo) and (hi is None or d <= hi)
        mrun, carry = None, (None, None)
        for tok in ORDER:
            if tok == 'q' and ok(1): qproj(n + 1)
            elif tok == 'f' and ok(-LAG): o = fin((lb[1 - par][...], ab[1 - par][...]) if LAG else carry)
            elif tok == 'O' and ok(-LAG): outproj(n - LAG, o)
            elif tok[0] == 'k' and ok(1): mrun = qk_chunk(n + 1, 1 - par, int(tok[1:]), mrun)
            elif tok == 'm' and ok(1): qk_fin(1 - par, mrun)
            elif tok[0] == 'p' and ok(0): carry = pv_chunk(n, par, int(tok[1:]), carry)
            elif tok == 's' and ok(0): stash(par, carry)

    pieces = []
    n0 = 0
    for cnt, iters in PHASES:
        for _ in range(iters):
            pieces.append((n0, cnt))
            n0 += cnt
    assert n0 == N
    nx = sum(1 for cnt, iters in PHASES if iters == 1 and cnt == 1)

    def fence():
        pl.semaphore_signal(sem_f, 1)
        pl.semaphore_wait(sem_f, 1)

    issue = []
    for i, (n0, cnt) in enumerate(pieces):
        if n0 % B == 0:
            issue.append(wq_copy(n0 // B))
        if n0 < nx:
            issue.append(x_copy(n0, 1))
        elif n0 == nx:
            issue.append(x_copy(nx, B - nx))
        if i > 0 and pieces[i - 1][1] == 1:
            issue.append(v_copy(*pieces[i - 1], i - 1))
        issue.append(k_copy(n0, cnt, i))
        if cnt > 1:
            issue.append(v_copy(n0, cnt, i))
        if n0 == 1 or (n0 > 0 and n0 % B == 0):
            issue.append(wo_copy(n0 // B))
    for c in issue:
        c.start()
        fence()
    acc_s[...] = jnp.zeros(acc_s.shape, F32)

    i0 = 0
    for cnt, iters in PHASES:
        n0 = pieces[i0][0]
        if i0 > 0 and pieces[i0 - 1][1] == 1:
            v_copy(*pieces[i0 - 1], i0 - 1).wait()
        if n0 == nx:
            x_copy(nx, B - nx).wait()
        if cnt == 1:
            assert iters == 1
            if n0 == 0:
                wq_copy(0).wait()
            if n0 == 1:
                wo_copy(0).wait()
            x_copy(n0, 1).wait()
            k_copy(n0, 1, i0).wait()
            slot(n0 - 1, (n0 - 1) % 2, lo=1 - n0)
        else:
            def body(it, c, cnt=cnt, n0=n0, i0=i0):
                n = n0 + it * cnt
                k_copy(n, cnt, i0 + it).wait()
                v_copy(n, cnt, i0 + it).wait()

                def new_head():
                    wq_copy(n // B).wait()
                    wo_copy(n // B).wait()
                if cnt == B:
                    new_head()
                else:
                    pl.when(n % B == 0)(new_head)
                for u in range(cnt):
                    slot(n + u - 1, (n0 + u - 1) % 2)
                return c
            lax.fori_loop(0, iters, body, 0)
        i0 += iters
    nb = B - 1 - LAG
    out_copy(0, nb, 0).start()
    for n in range(N - 1, N + LAG):
        slot(n, n % 2, hi=N - 1 - n)
    out_copy(nb, B - nb, 1).start()
    out_copy(0, nb, 0).wait()
    out_copy(nb, B - nb, 1).wait()


@jax.jit
def pallas_standalone__gqa_block_cached__near_ridge_kernel(x, k_cache, v_cache, wq, wo):
    B, Sq, D = x.shape
    _, Hkv, Sk, Dh = k_cache.shape
    Hq = wq.shape[1] // Dh
    rep = Hq // Hkv
    R, G = rep * Sq, rep * Dh
    npieces = sum(it for _, it in PHASES)
    any_spec = pl.BlockSpec(memory_space=pl.ANY)
    vm = pltpu.VMEM
    return pl.pallas_call(
        functools.partial(_kernel, B=B, Hkv=Hkv, Sq=Sq, Sk=Sk, rep=rep, Dh=Dh, qscale=Dh ** -0.5 * LOG2E),
        in_specs=[any_spec] * 5,
        out_specs=any_spec,
        out_shape=jax.ShapeDtypeStruct((B, Sq, D), x.dtype),
        scratch_shapes=[
            vm((B, Sq, D), BF16), vm((Hkv, D, G), BF16), vm((Hkv, G, D), BF16),
            vm((B * Hkv, Sk, Dh), BF16), vm((B * Hkv, Sk, Dh), BF16),
            vm((R, Dh), BF16),
            vm((R, Sk), F32), vm((R, Sk), F32),
            vm((R, 128), F32), vm((R, 128), F32),
            vm((R, Dh), F32), vm((R, Dh), F32),
            vm((R, 128), F32), vm((R, 128), F32),
            vm((B, Sq, D), F32), vm((B, Sq, D), BF16),
            pltpu.SemaphoreType.DMA((B,)), pltpu.SemaphoreType.DMA((Hkv,)), pltpu.SemaphoreType.DMA((Hkv,)),
            pltpu.SemaphoreType.DMA((npieces,)), pltpu.SemaphoreType.DMA((npieces,)), pltpu.SemaphoreType.DMA((2,)),
            pltpu.SemaphoreType.REGULAR,
        ],
        compiler_params=pltpu.CompilerParams(vmem_limit_bytes=100 * 1024 * 1024, disable_bounds_checks=bool(NOBC)),
    )(x, k_cache, v_cache, wq, wo)
```

```python
import jax
import jax.numpy as jnp
from jax import lax
import jax.experimental.pallas as pl
import jax.experimental.pallas.tpu as pltpu

LOG2E = 1.4426950408889634
LANES = 128
CHUNK = 512
PIECE = 4
UNROLL = 12
X_FIRST = 2
F32 = jnp.float32
BF16 = jnp.bfloat16
CONTRACT_LAST = (((1,), (1,)), ((), ()))


def _kernel(x_hbm, k_hbm, v_hbm, wq_hbm, wo_hbm, out_hbm,
            x_s, wq_s, wo_s, k_s, v_s, q_s, s0, s1, m0, m1, acc0, acc1, l0, l1, y_s, out_s,
            sem_in, sem_out, sem_fence):
    B, Sq, D = x_s.shape
    N, Sk, Dh = k_s.shape
    R = q_s.shape[1]
    rep, H = R // Sq, N // B
    G = rep * Dh
    s_buf, m_buf, acc_buf, l_buf = (s0, s1), (m0, m1), (acc0, acc1), (l0, l1)

    sem_x, sem_wq, sem_wo, sem_k = 0, 2, 2 + H, 2 + 2 * H
    sem_v = sem_k + N // PIECE

    def x_copy(b0, nb, i):
        return pltpu.make_async_copy(x_hbm.at[pl.ds(b0, nb)], x_s.at[pl.ds(b0, nb)], sem_in.at[sem_x + i])

    def wq_copy(h):
        return pltpu.make_async_copy(wq_hbm.at[:, pl.ds(h * G, G)], wq_s.at[h], sem_in.at[sem_wq + h])

    def wo_copy(h):
        rows = pl.ds(pl.multiple_of(h * G, G), G)
        return pltpu.make_async_copy(wo_hbm.at[rows], wo_s.at[h], sem_in.at[sem_wo + h])

    def kv_copy(hbm, buf, n, cnt, sem):
        return pltpu.make_async_copy(hbm.at[pl.ds(n % B, cnt), n // B], buf.at[pl.ds(n, cnt)], sem_in.at[sem])

    def k_copy(n):
        return kv_copy(k_hbm, k_s, n, PIECE, sem_k + n // PIECE)

    def v_copy(n):
        return kv_copy(v_hbm, v_s, n, PIECE, sem_v + n // PIECE)

    def out_copy(b0, nb, i):
        return pltpu.make_async_copy(out_s.at[pl.ds(b0, nb)], out_hbm.at[pl.ds(b0, nb)], sem_out.at[i])

    def fence():
        pl.semaphore_signal(sem_fence, 1)
        pl.semaphore_wait(sem_fence, 1)

    def q_proj(h, b0, nb):
        x = x_s[b0:b0 + nb].reshape(nb * Sq, D)
        q = jnp.dot(x, wq_s[h], preferred_element_type=F32)
        q = (q * (Dh ** -0.5 * LOG2E)).astype(BF16)
        for b in range(nb):
            for r in range(rep):
                q_s[h * B + b0 + b, r * Sq:(r + 1) * Sq, :] = q[b * Sq:(b + 1) * Sq, r * Dh:(r + 1) * Dh]

    def scores(n, slot):
        m = None
        for c in range(0, Sk, CHUNK):
            s = lax.dot_general(q_s[n], k_s[n, c:c + CHUNK, :], CONTRACT_LAST, preferred_element_type=F32)
            s_buf[slot][:, c:c + CHUNK] = s
            for t in range(0, CHUNK, LANES):
                m = s[:, t:t + LANES] if m is None else jnp.maximum(m, s[:, t:t + LANES])
        m_buf[slot][...] = jnp.broadcast_to(jnp.max(m, axis=1, keepdims=True), (R, LANES))

    def attend(n, slot, midway=None):
        l = acc = None
        for c in range(0, Sk, CHUNK):
            if midway is not None and c == Sk // 2:
                midway()
            m = m_buf[slot][...]
            ps = [jnp.exp2(s_buf[slot][:, t:t + LANES] - m) for t in range(c, c + CHUNK, LANES)]
            for p in ps:
                l = p if l is None else l + p
            p = jnp.concatenate(ps, axis=1).astype(BF16)
            o = jnp.dot(p, v_s[n, c:c + CHUNK, :], preferred_element_type=F32)
            acc = o if acc is None else acc + o
        l_buf[slot][...] = l
        acc_buf[slot][...] = acc

    def out_proj(n, slot, last=False):
        l = jnp.sum(l_buf[slot][...], axis=1, keepdims=True)
        o = acc_buf[slot][...] * pl.reciprocal(l, full_range=False)
        o = jnp.concatenate([o[r * Sq:(r + 1) * Sq] for r in range(rep)], axis=1).astype(BF16)
        y = y_s[n % B]
        if last:
            for r in range(rep):
                y = y + jnp.dot(o[:, r * Dh:(r + 1) * Dh], wo_s[n // B, r * Dh:(r + 1) * Dh, :],
                                preferred_element_type=F32)
        else:
            y = y + jnp.dot(o, wo_s[n // B], preferred_element_type=F32)
            y_s[n % B] = y
        out_s[n % B] = y.astype(BF16)

    x_first, x_rest = x_copy(0, X_FIRST, 0), x_copy(X_FIRST, B - X_FIRST, 1)
    v_first = kv_copy(v_hbm, v_s, 0, PIECE - 1, sem_v)
    v_rest = kv_copy(v_hbm, v_s, PIECE - 1, 1, sem_v + N // PIECE)
    copies = [wq_copy(0), x_first, x_rest] + [wq_copy(h) for h in range(1, H)]
    copies += [k_copy(0), v_first, wo_copy(0), v_rest]
    for n in range(PIECE, N, PIECE):
        copies += [k_copy(n), v_copy(n)] + ([wo_copy(n // B)] if n % B == 0 else [])
    for copy in copies:
        copy.start()
        fence()
    y_s[...] = jnp.zeros(y_s.shape, F32)

    wq_copy(0).wait()
    x_first.wait()
    q_proj(0, 0, X_FIRST)
    fence()
    x_rest.wait()
    q_proj(0, X_FIRST, B - X_FIRST)
    fence()
    for h in range(1, H):
        wq_copy(h).wait()
        if h == H - 1:
            k_copy(0).wait()
            v_first.wait()
            wo_copy(0).wait()
        q_proj(h, 0, B)

    for n in range(PIECE):
        if n >= 1:
            attend(n - 1, (n - 1) % 2)
        scores(n, n % 2)
        if n >= 2:
            out_proj(n - 2, n % 2)
    v_rest.wait()

    def steps(it, carry):
        for u in range(UNROLL):
            n = PIECE + it * UNROLL + u
            attend(n - 1, (u - 1) % 2)
            if u % PIECE == 0:
                k_copy(n).wait()
                v_copy(n).wait()
                pl.when(n % B == 0)(lambda: wo_copy(n // B).wait())
            scores(n, u % 2)
            out_proj(n - 2, u % 2)
        return carry

    lax.fori_loop(0, (N - PIECE) // UNROLL, steps, None)

    def second_last():
        out_proj(N - 2, N % 2)
        out_copy(B - 2, 1, 1).start()

    out_copy(0, B - 2, 0).start()
    attend(N - 1, (N - 1) % 2, midway=second_last)
    out_proj(N - 1, (N - 1) % 2, last=True)
    out_copy(B - 1, 1, 2).start()
    out_copy(0, B - 2, 0).wait()
    out_copy(B - 2, 1, 1).wait()
    out_copy(B - 1, 1, 2).wait()


@jax.jit
def pallas_standalone__gqa_block_cached__near_ridge_kernel(
    x: jax.Array,
    k_cache: jax.Array,
    v_cache: jax.Array,
    wq: jax.Array,
    wo: jax.Array,
):
    B, Sq, D = x.shape
    _, Hkv, Sk, Dh = k_cache.shape
    N = B * Hkv
    G = wq.shape[1] // Hkv
    R = G // Dh * Sq
    assert Dh == LANES and Sk % (2 * CHUNK) == 0 and B > X_FIRST
    assert B % PIECE == 0 and UNROLL % PIECE == 0 and (N - PIECE) % UNROLL == 0

    vmem, dma = pltpu.VMEM, pltpu.SemaphoreType.DMA
    return pl.pallas_call(
        _kernel,
        in_specs=[pl.BlockSpec(memory_space=pl.ANY)] * 5,
        out_specs=pl.BlockSpec(memory_space=pl.ANY),
        out_shape=jax.ShapeDtypeStruct((B, Sq, D), x.dtype),
        scratch_shapes=[
            vmem((B, Sq, D), BF16),
            vmem((Hkv, D, G), BF16),
            vmem((Hkv, G, D), BF16),
            vmem((N, Sk, Dh), BF16),
            vmem((N, Sk, Dh), BF16),
            vmem((N, R, Dh), BF16),
            vmem((R, Sk), F32), vmem((R, Sk), F32),
            vmem((R, LANES), F32), vmem((R, LANES), F32),
            vmem((R, Dh), F32), vmem((R, Dh), F32),
            vmem((R, LANES), F32), vmem((R, LANES), F32),
            vmem((B, Sq, D), F32),
            vmem((B, Sq, D), x.dtype),
            dma((2 + 2 * Hkv + 2 * (N // PIECE) + 1,)),
            dma((3,)),
            pltpu.SemaphoreType.REGULAR,
        ],
        compiler_params=pltpu.CompilerParams(
            vmem_limit_bytes=100 * 1024 * 1024,
            flags={
                "XLA_TPU_FORCE_LP_LLO_SCHEDULER": True,
                "XLA_TPU_RESCHEDULE_DMA_DONES": True,
            },
        ),
    )(x, k_cache, v_cache, wq, wo)
```

```python
import functools

import jax
import jax.numpy as jnp
from jax import lax
import jax.experimental.pallas as pl
import jax.experimental.pallas.tpu as pltpu

LOG2E = 1.4426950408889634
LANES = 128
CHUNK = 512
PIECE = 4
UNROLL = 12
X_FIRST = 2
F32 = jnp.float32
BF16 = jnp.bfloat16
CONTRACT_LAST = (((1,), (1,)), ((), ()))


def _block(x_hbm, k_hbm, v_hbm, wq_hbm, wo_hbm,
           x_s, wq_s, wo_s, k_s, v_s, q_s, s0, s1, m0, m1, acc0, acc1, l0, l1, y_s, out_s,
           out_copies, sem_in, sem_fence):
    B, Sq, D = x_s.shape
    N, Sk, Dh = k_s.shape
    R = q_s.shape[1]
    rep, H = R // Sq, N // B
    G = rep * Dh
    s_buf, m_buf, acc_buf, l_buf = (s0, s1), (m0, m1), (acc0, acc1), (l0, l1)

    sem_x, sem_wq, sem_wo, sem_k = 0, 2, 2 + H, 2 + 2 * H
    sem_v = sem_k + N // PIECE

    def x_copy(b0, nb, i):
        return pltpu.make_async_copy(x_hbm.at[pl.ds(b0, nb)], x_s.at[pl.ds(b0, nb)], sem_in.at[sem_x + i])

    def wq_copy(h):
        return pltpu.make_async_copy(wq_hbm.at[:, pl.ds(h * G, G)], wq_s.at[h], sem_in.at[sem_wq + h])

    def wo_copy(h):
        rows = pl.ds(pl.multiple_of(h * G, G), G)
        return pltpu.make_async_copy(wo_hbm.at[rows], wo_s.at[h], sem_in.at[sem_wo + h])

    def kv_copy(hbm, buf, n, cnt, sem):
        return pltpu.make_async_copy(hbm.at[pl.ds(n % B, cnt), n // B], buf.at[pl.ds(n, cnt)], sem_in.at[sem])

    def k_copy(n):
        return kv_copy(k_hbm, k_s, n, PIECE, sem_k + n // PIECE)

    def v_copy(n):
        return kv_copy(v_hbm, v_s, n, PIECE, sem_v + n // PIECE)

    def fence():
        pl.semaphore_signal(sem_fence, 1)
        pl.semaphore_wait(sem_fence, 1)

    def q_proj(h, b0, nb):
        x = x_s[b0:b0 + nb].reshape(nb * Sq, D)
        q = jnp.dot(x, wq_s[h], preferred_element_type=F32)
        q = (q * (Dh ** -0.5 * LOG2E)).astype(BF16)
        for b in range(nb):
            for r in range(rep):
                q_s[h * B + b0 + b, r * Sq:(r + 1) * Sq, :] = q[b * Sq:(b + 1) * Sq, r * Dh:(r + 1) * Dh]

    def scores(n, slot):
        m = None
        for c in range(0, Sk, CHUNK):
            s = lax.dot_general(q_s[n], k_s[n, c:c + CHUNK, :], CONTRACT_LAST, preferred_element_type=F32)
            s_buf[slot][:, c:c + CHUNK] = s
            for t in range(0, CHUNK, LANES):
                m = s[:, t:t + LANES] if m is None else jnp.maximum(m, s[:, t:t + LANES])
        m_buf[slot][...] = jnp.broadcast_to(jnp.max(m, axis=1, keepdims=True), (R, LANES))

    def attend(n, slot, midway=None):
        l = acc = None
        for c in range(0, Sk, CHUNK):
            if midway is not None and c == Sk // 2:
                midway()
            m = m_buf[slot][...]
            ps = [jnp.exp2(s_buf[slot][:, t:t + LANES] - m) for t in range(c, c + CHUNK, LANES)]
            for p in ps:
                l = p if l is None else l + p
            p = jnp.concatenate(ps, axis=1).astype(BF16)
            o = jnp.dot(p, v_s[n, c:c + CHUNK, :], preferred_element_type=F32)
            acc = o if acc is None else acc + o
        l_buf[slot][...] = l
        acc_buf[slot][...] = acc

    def out_proj(n, slot, last=False):
        l = jnp.sum(l_buf[slot][...], axis=1, keepdims=True)
        o = acc_buf[slot][...] * pl.reciprocal(l, full_range=False)
        o = jnp.concatenate([o[r * Sq:(r + 1) * Sq] for r in range(rep)], axis=1).astype(BF16)
        y = y_s[n % B]
        if last:
            for r in range(rep):
                y = y + jnp.dot(o[:, r * Dh:(r + 1) * Dh], wo_s[n // B, r * Dh:(r + 1) * Dh, :],
                                preferred_element_type=F32)
        else:
            y = y + jnp.dot(o, wo_s[n // B], preferred_element_type=F32)
            y_s[n % B] = y
        out_s[n % B] = y.astype(BF16)

    x_first, x_rest = x_copy(0, X_FIRST, 0), x_copy(X_FIRST, B - X_FIRST, 1)
    v_first = kv_copy(v_hbm, v_s, 0, PIECE - 1, sem_v)
    v_rest = kv_copy(v_hbm, v_s, PIECE - 1, 1, sem_v + N // PIECE)
    copies = [wq_copy(0), x_first, x_rest] + [wq_copy(h) for h in range(1, H)]
    copies += [k_copy(0), v_first, wo_copy(0), v_rest]
    for n in range(PIECE, N, PIECE):
        copies += [k_copy(n), v_copy(n)] + ([wo_copy(n // B)] if n % B == 0 else [])
    for copy in copies:
        copy.start()
        fence()
    y_s[...] = jnp.zeros(y_s.shape, F32)

    wq_copy(0).wait()
    x_first.wait()
    q_proj(0, 0, X_FIRST)
    fence()
    x_rest.wait()
    q_proj(0, X_FIRST, B - X_FIRST)
    fence()
    for h in range(1, H):
        wq_copy(h).wait()
        if h == H - 1:
            k_copy(0).wait()
            v_first.wait()
            wo_copy(0).wait()
        q_proj(h, 0, B)

    for n in range(PIECE):
        if n >= 1:
            attend(n - 1, (n - 1) % 2)
        scores(n, n % 2)
        if n >= 2:
            out_proj(n - 2, n % 2)
    v_rest.wait()

    def steps(it, carry):
        for u in range(UNROLL):
            n = PIECE + it * UNROLL + u
            attend(n - 1, (u - 1) % 2)
            if u % PIECE == 0:
                k_copy(n).wait()
                v_copy(n).wait()
                pl.when(n % B == 0)(lambda: wo_copy(n // B).wait())
            scores(n, u % 2)
            out_proj(n - 2, u % 2)
        return carry

    lax.fori_loop(0, (N - PIECE) // UNROLL, steps, None)

    def second_last():
        out_proj(N - 2, N % 2)
        out_copies[1].start()

    out_copies[0].start()
    attend(N - 1, (N - 1) % 2, midway=second_last)
    out_proj(N - 1, (N - 1) % 2, last=True)
    out_copies[2].start()


def _kernel(x_hbm, k_hbm, v_hbm, wq_hbm, wo_hbm, out_hbm, *scratch):
    *buffers, out_s, sem_out = scratch
    B, Hkv = k_hbm.shape[:2]
    out_copies = [
        pltpu.make_async_copy(out_s.at[pl.ds(b0, nb)], out_hbm.at[pl.ds(b0, nb)], sem_out.at[i])
        for i, (b0, nb) in enumerate(((0, B - 2), (B - 2, 1), (B - 1, 1)))
    ]
    pl.run_scoped(
        functools.partial(_block, x_hbm, k_hbm, v_hbm, wq_hbm, wo_hbm, *buffers, out_s, out_copies),
        pltpu.SemaphoreType.DMA((2 + 2 * Hkv + 2 * (B * Hkv // PIECE) + 1,)),
        pltpu.SemaphoreType.REGULAR,
    )
    for copy in out_copies:
        copy.wait()


@jax.jit
def pallas_standalone__gqa_block_cached__near_ridge_kernel(
    x: jax.Array,
    k_cache: jax.Array,
    v_cache: jax.Array,
    wq: jax.Array,
    wo: jax.Array,
):
    B, Sq, D = x.shape
    _, Hkv, Sk, Dh = k_cache.shape
    N = B * Hkv
    G = wq.shape[1] // Hkv
    R = G // Dh * Sq
    assert Dh == LANES and Sk % (2 * CHUNK) == 0 and B > X_FIRST
    assert B % PIECE == 0 and UNROLL % PIECE == 0 and (N - PIECE) % UNROLL == 0

    vmem = pltpu.VMEM
    return pl.pallas_call(
        _kernel,
        in_specs=[pl.BlockSpec(memory_space=pl.ANY)] * 5,
        out_specs=pl.BlockSpec(memory_space=pl.ANY),
        out_shape=jax.ShapeDtypeStruct((B, Sq, D), x.dtype),
        scratch_shapes=[
            vmem((B, Sq, D), BF16),
            vmem((Hkv, D, G), BF16),
            vmem((Hkv, G, D), BF16),
            vmem((N, Sk, Dh), BF16),
            vmem((N, Sk, Dh), BF16),
            vmem((N, R, Dh), BF16),
            vmem((R, Sk), F32), vmem((R, Sk), F32),
            vmem((R, LANES), F32), vmem((R, LANES), F32),
            vmem((R, Dh), F32), vmem((R, Dh), F32),
            vmem((R, LANES), F32), vmem((R, LANES), F32),
            vmem((B, Sq, D), F32),
            vmem((B, Sq, D), x.dtype),
            pltpu.SemaphoreType.DMA((3,)),
        ],
        compiler_params=pltpu.CompilerParams(
            vmem_limit_bytes=100 * 1024 * 1024,
            flags={
                "XLA_TPU_FORCE_LP_LLO_SCHEDULER": True,
                "XLA_TPU_RESCHEDULE_DMA_DONES": True,
            },
        ),
    )(x, k_cache, v_cache, wq, wo)
```
